```python
import os as _os
_os.environ.setdefault("JAX_PLATFORMS", "cpu")
import jax
import jax.numpy as jnp

def _softmax(x, axis=-1):
    return jax.nn.softmax(x, axis=axis)
def _gelu(x):
    return jax.nn.gelu(x, approximate=True)
def _silu(x):
    return jax.nn.silu(x)
def _sigmoid(x):
    return jax.nn.sigmoid(x)
def _layernorm(x, axis=-1, eps=1e-5):
    m = jnp.mean(x, axis=axis, keepdims=True)
    v = jnp.var(x, axis=axis, keepdims=True)
    return (x - m) / jnp.sqrt(v + eps)
def _scatter_add(tgt, idx, src, axis=0):
    return tgt.at[idx].add(src)
def _segment_sum(src, seg, n):
    return jax.ops.segment_sum(src, seg, n)
class _Rng:
    def __init__(self, key):
        self._k = key
    def _next(self):
        self._k, sub = jax.random.split(self._k)
        return sub
    def normal(self, shape):
        return jax.random.normal(self._next(), shape, dtype=jnp.bfloat16)
    def randint(self, lo, hi, shape):
        return jax.random.randint(self._next(), shape, lo, hi, dtype=jnp.int32)
    def uniform(self, shape, lo=0.0, hi=1.0):
        return jax.random.uniform(self._next(), shape, jnp.bfloat16, lo, hi)
    def permutation(self, n):
        return jax.random.permutation(self._next(), n)


kernel_name = 'sequential_preLN__sliding_local_dilated__dense_activation_mish__prompt'

def setup_inputs():
    _rng = _Rng(jax.random.key(int.from_bytes(__import__("os").urandom(4), "little")))
    _w = (lambda a: (lambda t: t.astype(jnp.bfloat16) if jnp.issubdtype(t.dtype, jnp.floating) else t)(jnp.asarray(a)))
    def _A_setup():
        B, S, D = 1, 2048, 512
        return {
            "x": _w((lambda *s: _rng.normal(s) * 0.05)(B, S, D)),
            "wqkv": _w((lambda *s: _rng.normal(s) * 0.05)(D, 3 * D)),
            "wo": _w((lambda *s: _rng.normal(s) * 0.05)(D, D)),
        }
    _A_in = _A_setup()

    def _B_setup():
        B, S, D, F = 1, 2048, 512, 1376
        return {
            "x": _w((lambda *s: _rng.normal(s) * 0.05)(B, S, D)),
            "w1": _w((lambda *s: _rng.normal(s) * 1.6)(D, F) * (D ** -0.5)),
            "b1": _w((lambda *s: _rng.normal(s) * 0.1)(F)),
            "w2": _w((lambda *s: _rng.normal(s) * 0.1)(F, D) * (F ** -0.5)),
        }
    _B_in = _B_setup()

    return {
        "A_x": _A_in["x"],
        "A_wqkv": _A_in["wqkv"],
        "A_wo": _A_in["wo"],
        "B_x": _B_in["x"],
        "B_w1": _B_in["w1"],
        "B_b1": _B_in["b1"],
        "B_w2": _B_in["w2"],
    }

def reference(A_x, A_wqkv, A_wo, B_x, B_w1, B_b1, B_w2):
    def _A_ref(x, wqkv, wo):
        B, S, D = x.shape
        H = 32; Dh = D // H
        W, dil = 8, 2
        qkv = (lambda x, *d: x.transpose(*d))((x @ wqkv).reshape(B, S, 3, H, Dh), 2, 0, 3, 1, 4)
        q, k, v = qkv[0], qkv[1], qkv[2]
        scale = Dh ** -0.5
        pos = jnp.arange(S)
        off = jnp.arange(W) * dil
        idx = pos[:, None] - off[None, :]
        mask = idx >= 0
        idx_c = jnp.where(mask, idx, 0).reshape(-1)
        kg = k[:, :, idx_c, :].reshape(B, H, S, W, Dh)
        vg = v[:, :, idx_c, :].reshape(B, H, S, W, Dh)
        logits = jnp.einsum("bhsd,bhswd->bhsw", q, kg) * scale
        logits = jnp.where(mask[None, None, :, :], logits, -1e9)
        attn = _softmax(logits, axis=-1)
        o = jnp.einsum("bhsw,bhswd->bhsd", attn, vg)
        return (lambda x, *d: x.transpose(*d))(o, 0, 2, 1, 3).reshape(B, S, D) @ wo

    def _B_ref(x, w1, b1, w2):
        h = jnp.einsum("bsd,df->bsf", x, w1) + b1
        sp = jnp.log1p(jnp.exp(-jnp.abs(h))) + jnp.where(h > 0, h, jnp.zeros_like(h))
        act = h * jnp.tanh(sp)
        return jnp.einsum("bsf,fd->bsd", act, w2)

    x = A_x
    h = x + _A_ref(_layernorm(x, axis=-1), A_wqkv, A_wo)
    h2 = h + _B_ref(_layernorm(h, axis=-1), B_w1, B_b1, B_w2)
    return h2
```

```python
import functools, math, itertools
import numpy as np
import jax, jax.numpy as jnp
from jax import lax
import jax.experimental.pallas as pl
import jax.experimental.pallas.tpu as pltpu

D, H, DH, F = 512, 32, 16, 1376
FP = 1408
HALO = 16
LOG2E = 1.4426950408889634
f32, bf16, i32 = jnp.float32, jnp.bfloat16, jnp.int32
NT_DN = (((1,), (1,)), ((), ()))

def interleave(a, b):
    out = []
    na, nb = len(a), len(b)
    ia = ib = 0
    while ia < na or ib < nb:
        if ib >= nb or (ia < na and (ia + 0.5) * nb <= (ib + 0.5) * na):
            out.append(a[ia]); ia += 1
        else:
            out.append(b[ib]); ib += 1
    return out

def make(T=256, R=16, LR=16, order="Y", flags={"XLA_TPU_RESCHEDULE_DMA_DONES": True}, nobc=True, interpret=False, S=2048, fresh=False, rot3=False, dynst=False):
    NT = S // T
    NSEM = NT + 12 + 4 * 3 + 1 + 4 * NT
    def kernel(x_hbm, wqkv_hbm, wo_hbm, w1t_hbm, b1_hbm, w2_hbm, out_hbm,
               xb, wraw, wq, woraw, wop, w1b, w2b, b1r, bb, xn, qb, kb, vb, ob, hb, hn, act, outb, sem, zsem):
        z = pl.semaphore_read(zsem)
        ctr = itertools.count(1)
        def fz():
            return z * next(ctr) if fresh else 0
        def fzs():
            return z * next(ctr) if (fresh or dynst) else 0
        def sx(i): return i
        def swr(t): return NT + t
        def swo(c): return NT + 12 + c
        def sw1(c): return NT + 16 + c
        def sw2(c): return NT + 20 + c
        sb1 = NT + 24
        def sout(i, n): return NT + 25 + i * 4 + n
        x_cp = [pltpu.make_async_copy(x_hbm.at[i * T:(i + 1) * T, :], xb.at[0, i * T:(i + 1) * T, :], sem.at[sx(i)]) for i in range(NT)]
        wr_cp = [pltpu.make_async_copy(wqkv_hbm.at[:, t * 128:(t + 1) * 128], wraw.at[t], sem.at[swr(t)]) for t in range(12)]
        wo_cp = [pltpu.make_async_copy(wo_hbm.at[:, c * 128:(c + 1) * 128], woraw.at[c], sem.at[swo(c)]) for c in range(4)]
        w1_cp = [pltpu.make_async_copy(w1t_hbm.at[:, c * 128:(c + 1) * 128], w1b.at[0, c, 0:F, :], sem.at[sw1(c)]) for c in range(4)]
        w2_cp = [pltpu.make_async_copy(w2_hbm.at[:, c * 128:(c + 1) * 128], w2b.at[0, c, 0:F, :], sem.at[sw2(c)]) for c in range(4)]
        b1_cp = pltpu.make_async_copy(b1_hbm, b1r, sem.at[sb1])
        out_cp = [[pltpu.make_async_copy(outb.at[0, n, i * T:(i + 1) * T, :], out_hbm.at[i * T:(i + 1) * T, n * 128:(n + 1) * 128], sem.at[sout(i, n)])
                   for n in range(4)] for i in range(NT)]
        part_order = (1, 2, 0)
        x_cp[0].start()
        for p_ in part_order:
            for a in range(4):
                wr_cp[p_ * 4 + a].start()
        if NT > 1: x_cp[1].start()
        for c in range(4): wo_cp[c].start()
        b1_cp.start()
        for c in range(4): w1_cp[c].start()
        for c in range(4): w2_cp[c].start()
        for i in range(2, NT): x_cp[i].start()

        zf = jnp.zeros((4, HALO, 128), f32)
        kb[fzs(), :, 0:HALO, :] = zf
        vb[fzs(), :, 0:HALO, :] = zf
        zb = jnp.zeros((4, FP - F, 128), bf16)
        w1b[0, :, F:FP, :] = zb
        w2b[0, :, F:FP, :] = zb

        wraw_i = wraw.bitcast(i32); woraw_i = woraw.bitcast(i32); w1_i = w1b.bitcast(i32); w2_i = w2b.bitcast(i32)
        outb_i = outb.bitcast(i32)
        asbf = lambda v: pltpu.bitcast(v, bf16)
        def pack(v):
            return pltpu.bitcast(v.astype(bf16), i32)

        rr = lax.broadcasted_iota(i32, (128, 128), 0); cc = lax.broadcasted_iota(i32, (128, 128), 1)
        P = jnp.where(cc == (rr % 8) * 16 + rr // 8, 1.0, 0.0).astype(bf16)

        def perm_wq(part, ap):
            def f():
                rs = []
                for a in (2 * ap, 2 * ap + 1):
                    t = part * 4 + a
                    wr_cp[t].wait()
                    rs.append(lax.dot_general(P, asbf(wraw_i[t]), NT_DN, preferred_element_type=f32))
                w = wq.at[fzs()]
                for d in range(16):
                    v = jnp.concatenate([rs[0][d * 8:(d + 1) * 8], rs[1][d * 8:(d + 1) * 8]], axis=0)
                    pv = pack(v)
                    row = (part * D + d * 32 + ap * 16) // 2
                    for kt in range(4):
                        w[kt, row:row + 8, :] = pv[:, kt * 128:(kt + 1) * 128]
            return f
        def perm_wo(ap):
            def f():
                rs = []
                if ap == 0:
                    for c in range(4): wo_cp[c].wait()
                for a in (2 * ap, 2 * ap + 1):
                    rhs = jnp.concatenate([asbf(woraw_i[c, a * 64:(a + 1) * 64, :]) for c in range(4)], axis=1)
                    rs.append(jnp.dot(P, rhs, preferred_element_type=f32))
                w = wop.at[fzs()]
                for d in range(16):
                    v = jnp.concatenate([rs[0][d * 8:(d + 1) * 8], rs[1][d * 8:(d + 1) * 8]], axis=0)
                    pv = pack(v)
                    row = (d * 32 + ap * 16) // 2
                    for c in range(4):
                        w[c, row:row + 8, :] = pv[:, c * 128:(c + 1) * 128]
            return f
        def prep_b1():
            b1_cp.wait()
            bv = b1r[...].astype(f32)[None, :]
            w = bb.at[fzs()]
            w[:, FP - 128:FP] = jnp.zeros((8, 128), f32)
            w[:, 0:F] = jnp.broadcast_to(bv, (8, F))

        def ln_vals(xf):
            m = jnp.mean(xf, axis=-1, keepdims=True)
            c = xf - m
            v = jnp.mean(c * c, axis=-1, keepdims=True)
            return c * lax.rsqrt(v + 1e-5)
        def store_lhs(buf, r0, rows, val):
            pv = pack(val)
            for kt in range(val.shape[1] // 128):
                buf[kt, r0 // 2:(r0 + rows) // 2, :] = pv[:, kt * 128:(kt + 1) * 128]
        def load_lhs(buf, nk):
            return jnp.concatenate([asbf(buf[kt]) for kt in range(nk)], axis=1)
        def ln1(i, c):
            def f():
                g = i * T + c * LR
                if c == 0: x_cp[i].wait()
                store_lhs(xn.at[fzs(), i % 2], c * LR, LR, ln_vals(xb[fz(), g:g + LR, :].astype(f32)))
            return f
        def qkv(i, n):
            def f():
                part = part_order[n // 4]; t = n % 4
                row = (part * D + t * 128) // 2
                w = wq.at[fz()]
                rhs = jnp.concatenate([asbf(w[kt, row:row + 64, :]) for kt in range(4)], axis=1)
                r = lax.dot_general(load_lhs(xn.at[fz(), i % 2], 4), rhs, NT_DN, preferred_element_type=f32)
                g = i * T
                if part == 0:
                    qb[fzs(), t, g:g + T, :] = r * (0.25 * LOG2E)
                elif part == 1:
                    kb[fzs(), t, HALO + g:HALO + g + T, :] = r
                else:
                    vb[fzs(), t, HALO + g:HALO + g + T, :] = r
            return f
        def attn(i, c):
            def f():
                g = i * T + c * R
                qr, kr, vr = qb.at[fz()], kb.at[fz()], vb.at[fz()]
                q = [qr[t, g:g + R, :] for t in range(4)]
                s = []
                for j in range(8):
                    a = HALO + g - 2 * j
                    acc = q[0] * kr[0, a:a + R, :]
                    for t in range(1, 4):
                        acc = acc + q[t] * kr[t, a:a + R, :]
                    if rot3:
                        acc = (acc + pltpu.roll(acc, 64, 1)) + (pltpu.roll(acc, 32, 1) + pltpu.roll(acc, 96, 1))
                    else:
                        acc = acc + pltpu.roll(acc, 64, 1)
                        acc = acc + pltpu.roll(acc, 32, 1)
                    if g < 14 and j > 0:
                        pos = g + lax.broadcasted_iota(i32, (R, 128), 0)
                        acc = jnp.where(pos >= 2 * j, acc, -1e9)
                    s.append(acc)
                m = s[0]
                for j in range(1, 8):
                    m = jnp.maximum(m, s[j])
                p = [jnp.exp2(sj - m) for sj in s]
                l = p[0]
                for j in range(1, 8):
                    l = l + p[j]
                inv = pl.reciprocal(l, approx=True)
                o = [None] * 4
                for j in range(8):
                    a = HALO + g - 2 * j
                    for t in range(4):
                        term = p[j] * vr[t, a:a + R, :]
                        o[t] = term if o[t] is None else o[t] + term
                w = ob.at[fzs(), i % 2]
                for t in range(4):
                    w[t, c * R // 2:(c + 1) * R // 2, :] = pack(o[t] * inv)
            return f
        def wo(i, n):
            def f():
                r = jnp.dot(load_lhs(ob.at[fz(), i % 2], 4), asbf(wop[fz(), n]), preferred_element_type=f32)
                g = i * T
                hb[fzs(), i % 2, :, n * 128:(n + 1) * 128] = r + xb[fz(), g:g + T, n * 128:(n + 1) * 128].astype(f32)
            return f
        def ln2(i, c):
            def f():
                store_lhs(hn.at[fzs()], c * LR, LR, ln_vals(hb[fz(), i % 2, c * LR:(c + 1) * LR, :]))
            return f
        def w1(i, n):
            def f():
                if i == 0 and n == 0:
                    for c in range(4): w1_cp[c].wait()
                w = w1_i.at[fz()]
                rhs = jnp.concatenate([asbf(w[kt, n * 64:(n + 1) * 64, :]) for kt in range(4)], axis=1)
                h1 = lax.dot_general(load_lhs(hn.at[fz()], 4), rhs, NT_DN, preferred_element_type=f32)
                h1 = h1 + jnp.concatenate([bb[fz(), :, n * 128:(n + 1) * 128]] * (T // 8), axis=0)
                e = jnp.exp2(jnp.minimum(h1, 20.0) * LOG2E)
                nn = e * (e + 2.0)
                a_ = h1 * nn * pl.reciprocal(nn + 2.0, approx=True)
                act[fzs(), n] = pack(a_)
            return f
        def w2(i, n):
            def f():
                if i == 0 and n == 0:
                    for c in range(4): w2_cp[c].wait()
                r = jnp.dot(load_lhs(act.at[fz()], 11), asbf(w2_i[fz(), n]), preferred_element_type=f32)
                g = i * T
                outb_i[fzs(), n, g // 2:(g + T) // 2, :] = pack(r + hb[fz(), i % 2, :, n * 128:(n + 1) * 128])
                out_cp[i][n].start()
            return f
        L = lambda fn, i, n: [fn(i, c) for c in range(n)] if 0 <= i < NT else []
        prog = []
        NC = T // R; NL = T // LR
        if order == "Y":
            q0 = L(qkv, 0, 12)
            pre = L(ln1, 0, NL)
            prog += [perm_wq(1, 0), perm_wq(1, 1)] + pre
            prog += q0[0:2] + [perm_wq(2, 0)] + q0[2:4] + [perm_wq(2, 1)] + q0[4:6] + [perm_wq(0, 0)] + q0[6:8] + [perm_wq(0, 1)] + q0[8:12]
            prog += L(ln1, 1, NL)
            prog += [perm_wo(0), perm_wo(1), prep_b1]
            prog += interleave(L(qkv, 1, 12), interleave(L(attn, 0, NC), L(ln1, 2, NL)))
            for i in range(NT):
                prog += L(wo, i, 4)
                if i + 2 < NT:
                    prog += interleave(L(qkv, i + 2, 12), L(ln2, i, NL))
                else:
                    prog += L(ln2, i, NL)
                prog += interleave(L(w1, i, 11) + L(w2, i, 4), interleave(L(attn, i + 1, NC), L(ln1, i + 3, NL)))
        elif order == "X":
            q0 = L(qkv, 0, 12)
            pre = L(ln1, 0, NL)
            prog += [perm_wq(1, 0), perm_wq(1, 1)] + pre
            prog += q0[0:2] + [perm_wq(2, 0)] + q0[2:4] + [perm_wq(2, 1)] + q0[4:6] + [perm_wq(0, 0)] + q0[6:8] + [perm_wq(0, 1)] + q0[8:12]
            prog += L(ln1, 1, NL)
            prog += [perm_wo(0), perm_wo(1), prep_b1]
            for i in range(NT):
                prog += interleave(L(qkv, i + 1, 12), L(attn, i, NC))
                prog += L(wo, i, 4) + L(ln2, i, NL) + L(w1, i, 11)
                prog += interleave(L(w2, i, 4), L(ln1, i + 2, NL))
        for p in prog:
            p()
        for i in range(NT):
            for n in range(4):
                out_cp[i][n].wait()

    @jax.jit
    def fn(A_x, A_wqkv, A_wo, B_x, B_w1, B_b1, B_w2):
        x = A_x.reshape(-1, D)
        hbm = pl.BlockSpec(memory_space=pltpu.HBM)
        cp = dict(vmem_limit_bytes=100 * 1024 * 1024, disable_bounds_checks=nobc)
        if flags: cp["flags"] = flags
        out = pl.pallas_call(
            kernel,
            in_specs=[hbm] * 6, out_specs=hbm,
            out_shape=jax.ShapeDtypeStruct((S, D), bf16),
            scratch_shapes=[
                pltpu.VMEM((1, S, D), bf16),
                pltpu.VMEM((12, D, 128), bf16),
                pltpu.VMEM((1, 4, 768, 128), i32),
                pltpu.VMEM((4, D, 128), bf16),
                pltpu.VMEM((1, 4, 256, 128), i32),
                pltpu.VMEM((1, 4, FP, 128), bf16),
                pltpu.VMEM((1, 4, FP, 128), bf16),
                pltpu.VMEM((F,), bf16),
                pltpu.VMEM((1, 8, FP), f32),
                pltpu.VMEM((1, 2, 4, T // 2, 128), i32),
                pltpu.VMEM((1, 4, S, 128), f32), pltpu.VMEM((1, 4, S + HALO, 128), f32), pltpu.VMEM((1, 4, S + HALO, 128), f32),
                pltpu.VMEM((1, 2, 4, T // 2, 128), i32),
                pltpu.VMEM((1, 2, T, D), f32),
                pltpu.VMEM((1, 4, T // 2, 128), i32),
                pltpu.VMEM((1, 11, T // 2, 128), i32),
                pltpu.VMEM((1, 4, S, 128), bf16),
                pltpu.SemaphoreType.DMA((NSEM,)), pltpu.SemaphoreType.REGULAR,
            ],
            compiler_params=pltpu.CompilerParams(**cp),
            name="fused_v5", interpret=interpret,
        )(x, A_wqkv, A_wo, B_w1.T, B_b1, B_w2)
        return out.reshape(1, S, D)
    return fn


pallas_sequential_preLN__sliding_local_dilated__dense_activation_mish__prompt_kernel = make()
```

```python
import jax
import jax.numpy as jnp
from jax import lax
import jax.experimental.pallas as pl
import jax.experimental.pallas.tpu as pltpu

S, D, H, DH, F = 2048, 512, 32, 16, 1376
FP = 1408
WIN, DIL = 8, 2
HALO = 16
T = 128
NT = S // T
LOG2E = 1.4426950408889634
f32, bf16, i32 = jnp.float32, jnp.bfloat16, jnp.int32
NT_DIMS = (((1,), (1,)), ((), ()))


def _interleave(a, b):
    out, ia, ib = [], 0, 0
    while ia < len(a) or ib < len(b):
        if ib >= len(b) or (ia < len(a) and (ia + 0.5) * len(b) <= (ib + 0.5) * len(a)):
            out.append(a[ia]); ia += 1
        else:
            out.append(b[ib]); ib += 1
    return out


def make(R=8, LR=16, qa=3, pa=(-1, 1, 0, 1, 0, 2, 3), w1s=5, w1pin=3, xg=(3, 4, 6, 10), xpin=9, x3pin=7,
         hold=3, nosc=True, kfine=False, escpos=5, interpret=False, nodma=False):
    xgroups = [(0, 1), (1, 2), (2, xg[0])] + list(zip(xg, list(xg[1:]) + [NT]))
    NX = len(xgroups)
    xg_of = {a: g for g, (a, _) in enumerate(xgroups)}
    S_X, S_W, S_WO, S_B1, S_W1A, S_W1B, S_W2, S_OUT, S_ESC = 0, NX, NX + 12, NX + 13, NX + 14, NX + 15, NX + 16, NX + 17, NX + 18
    NSEM = NX + 19
    W1R = w1s * 128
    NC, NL = T // R, T // LR

    def kernel(x_hbm, wqkv_hbm, wo_hbm, w1t_hbm, b1_hbm, w2_hbm, out_hbm,
               xb, wraw, wq, woraw, wop, w1b, w2b, b1r, bb, xn, qb, kb, vb, ob, hb, hn, act, outb, zf_, zi_, sem):
        mk = pltpu.make_async_copy
        asbf = lambda v: pltpu.bitcast(v, bf16)
        pack = lambda v: pltpu.bitcast(v.astype(bf16), i32)
        wraw_i, woraw_i, w1_i, w2_i, outb_i = (r.bitcast(i32) for r in (wraw, woraw, w1b, w2b, outb))

        def copies(nm, z=0):
            kind, idx = nm
            cols = lambda c: slice(c * 128, (c + 1) * 128)
            if kind == "x":
                a, b = xgroups[idx]
                return [mk(x_hbm.at[a * T:b * T, :], xb.at[a * T:b * T, :], sem.at[S_X + idx + z])]
            if kind == "w":
                return [mk(wqkv_hbm.at[:, cols(idx)], wraw.at[idx], sem.at[S_W + idx + z])]
            if kind == "wo":
                return [mk(wo_hbm.at[:, cols(c)], woraw.at[c], sem.at[S_WO + z]) for c in range(4)]
            if kind == "b1":
                return [mk(b1_hbm, b1r, sem.at[S_B1 + z])]
            if kind == "w1a":
                return [mk(w1t_hbm.at[0:W1R, cols(c)], w1b.at[c, 0:W1R, :], sem.at[S_W1A + z]) for c in range(4)]
            if kind == "w1b":
                return [mk(w1t_hbm.at[W1R:F, cols(c)], w1b.at[c, W1R:F, :], sem.at[S_W1B + z]) for c in range(4)]
            if kind == "w2":
                return [mk(w2_hbm.at[:, cols(c)], w2b.at[c, 0:F, :], sem.at[S_W2 + z]) for c in range(4)]

        def start(*names):
            if nodma: return
            for nm in names:
                for c in copies(nm):
                    c.start()

        pin = [0]

        def wait(*names):
            def f():
                z, pin[0] = pin[0], 0
                if nodma: return
                for nm in names:
                    for c in copies(nm, z):
                        c.wait()
            return f

        def pinned(task):
            def f():
                val = task()
                if nodma: return
                sign = lax.shift_right_logical(pltpu.bitcast(val, i32), 31).astype(f32)
                pin[0] = (jnp.max(sign) * 0.25).astype(i32)
            return f

        def pin_at(tasks, idx):
            return tasks[:idx] + [pinned(tasks[idx])] + tasks[idx + 1:]

        X = lambda g: ("x", g)
        k_t, v_t, q_t = [("w", 4 + a) for a in range(4)], [("w", 8 + a) for a in range(4)], [("w", a) for a in range(4)]
        first = [X(0)] + k_t
        start(*first[:escpos])
        zf_[...] = jnp.zeros((8, 128), f32)
        zi_[...] = jnp.zeros((8, 128), i32)
        esc = [mk(src, dst, sem.at[S_ESC]) for src, dst in (
            (zf_, hb.at[0, 0:8, 0:128]), (zi_, hn.at[0, 0, 0:8, :]), (zi_, act.at[0, 0, 0:8, :]),
            (zi_, xn.at[0, 0, 0:8, :]), (zf_, qb.at[0, 0:8, :]), (zf_, kb.at[0, 0:8, :]), (zf_, vb.at[0, 0:8, :]),
            (zi_, ob.at[0, 0, 0:8, :]), (zi_, wq.at[0, 0:8, :]), (zi_, wop.at[0, 0:8, :]), (zf_, bb.at[:, 0:128]))]
        for c in esc:
            c.start()
        start(*first[escpos:], X(1), *v_t, *q_t, X(2), ("wo", 0), ("b1", 0), ("w1a", 0), ("w1b", 0), ("w2", 0))
        start(*[X(g) for g in range(3, NX)])
        for c in esc:
            c.wait()

        rr = lax.broadcasted_iota(i32, (128, 128), 0)
        cc = lax.broadcasted_iota(i32, (128, 128), 1)
        P = jnp.where(cc == (rr % 8) * 16 + rr // 8, 1.0, 0.0).astype(bf16)

        def init():
            kb[:, 0:HALO, :] = jnp.zeros((4, HALO, 128), f32)
            vb[:, 0:HALO, :] = jnp.zeros((4, HALO, 128), f32)
            w1b[:, F:FP, :] = jnp.zeros((4, FP - F, 128), bf16)
            w2b[:, F:FP, :] = jnp.zeros((4, FP - F, 128), bf16)

        def perm_wq(part, ap):
            def f():
                rs = [lax.dot_general(P, asbf(wraw_i[part * 4 + a]), NT_DIMS, preferred_element_type=f32)
                      for a in (2 * ap, 2 * ap + 1)]
                for d in range(16):
                    pv = pack(jnp.concatenate([rs[0][d * 8:(d + 1) * 8], rs[1][d * 8:(d + 1) * 8]], axis=0))
                    row = (part * D + d * 32 + ap * 16) // 2
                    for kt in range(4):
                        wq[kt, row:row + 8, :] = pv[:, kt * 128:(kt + 1) * 128]
                return rs[1][120:128, 384:512]
            return f

        def perm_wo(c):
            def f():
                for dd in range(8):
                    a = woraw_i[c, pl.ds(dd, 16, stride=16), :]
                    b = woraw_i[c, pl.ds(8 + dd, 16, stride=16), :]
                    wop[c, 32 * dd:32 * dd + 16, :] = (a & 0xFFFF) | lax.shift_left(b, 16)
                    wop[c, 32 * dd + 16:32 * dd + 32, :] = lax.shift_right_logical(a, 16) | (b & jnp.int32(-65536))
            return f

        def prep_b1():
            bb[:, FP - 128:FP] = jnp.zeros((8, 128), f32)
            bb[:, 0:F] = jnp.broadcast_to(b1r[...].astype(f32)[None, :], (8, F))

        def layernorm(xf):
            m = jnp.mean(xf, axis=-1, keepdims=True)
            c = xf - m
            v = jnp.mean(c * c, axis=-1, keepdims=True)
            return c * lax.rsqrt(v + 1e-5)

        def store_lhs(buf, r0, rows, val):
            pv = pack(val)
            for kt in range(val.shape[1] // 128):
                buf[kt, r0 // 2:(r0 + rows) // 2, :] = pv[:, kt * 128:(kt + 1) * 128]

        def load_lhs(buf, nk):
            return jnp.concatenate([asbf(buf[kt]) for kt in range(nk)], axis=1)

        def ln1(i, c):
            def f():
                g = i * T + c * LR
                store_lhs(xn.at[i % 2], c * LR, LR, layernorm(xb[g:g + LR, :].astype(f32)))
            return f

        def qkv(i, n):
            def f():
                part, t = (1, 2, 0)[n // 4], n % 4
                row = (part * D + t * 128) // 2
                rhs = jnp.concatenate([asbf(wq[kt, row:row + 64, :]) for kt in range(4)], axis=1)
                r = lax.dot_general(load_lhs(xn.at[i % 2], 4), rhs, NT_DIMS, preferred_element_type=f32)
                g = i * T
                if part == 0:
                    qb[t, g:g + T, :] = r * (DH ** -0.5 * LOG2E)
                elif part == 1:
                    kb[t, HALO + g:HALO + g + T, :] = r
                else:
                    vb[t, HALO + g:HALO + g + T, :] = r
                return r[T - 8:T, :]
            return f

        def attn(i, c):
            def f():
                g = i * T + c * R
                q = [qb[t, g:g + R, :] for t in range(4)]
                s = []
                for j in range(WIN):
                    a = HALO + g - DIL * j
                    acc = q[0] * kb[0, a:a + R, :]
                    for t in range(1, 4):
                        acc = acc + q[t] * kb[t, a:a + R, :]
                    acc = (acc + pltpu.roll(acc, 64, 1)) + (pltpu.roll(acc, 32, 1) + pltpu.roll(acc, 96, 1))
                    if g < DIL * j:
                        pos = g + lax.broadcasted_iota(i32, (R, 128), 0)
                        acc = jnp.where(pos >= DIL * j, acc, -1e9)
                    s.append(acc)
                m = s[0]
                for j in range(1, WIN):
                    m = jnp.maximum(m, s[j])
                p = [jnp.exp2(sj - m) for sj in s]
                l = p[0]
                for j in range(1, WIN):
                    l = l + p[j]
                inv = pl.reciprocal(l, approx=True)
                o = [None] * 4
                for j in range(WIN):
                    a = HALO + g - DIL * j
                    for t in range(4):
                        term = p[j] * vb[t, a:a + R, :]
                        o[t] = term if o[t] is None else o[t] + term
                for t in range(4):
                    ob[i, t, c * R // 2:(c + 1) * R // 2, :] = pack(o[t] * inv)
            return f

        def wo(i, n):
            def f():
                r = jnp.dot(load_lhs(ob.at[i], 4), asbf(wop[n]), preferred_element_type=f32)
                g = i * T
                hb[i % 2, :, n * 128:(n + 1) * 128] = r + xb[g:g + T, n * 128:(n + 1) * 128].astype(f32)
                return r[T - 8:T, :]
            return f

        def ln2(i, c):
            def f():
                store_lhs(hn.at[i % 2], c * LR, LR, layernorm(hb[i % 2, c * LR:(c + 1) * LR, :]))
            return f

        def w1(i, n):
            def f():
                rhs = jnp.concatenate([asbf(w1_i[kt, n * 64:(n + 1) * 64, :]) for kt in range(4)], axis=1)
                h1 = lax.dot_general(load_lhs(hn.at[i % 2], 4), rhs, NT_DIMS, preferred_element_type=f32)
                h1 = h1 + jnp.concatenate([bb[:, n * 128:(n + 1) * 128]] * (T // 8), axis=0)
                e = jnp.exp2(jnp.minimum(h1, 10.0) * LOG2E)
                nn = e * (e + 2.0)
                a = h1 * nn * pl.reciprocal(nn + 2.0, approx=True)
                act[i % 2, n] = pack(a)
                return a[T - 8:T, :]
            return f

        out_started = []

        def w2(i, n):
            def f():
                r = jnp.dot(load_lhs(act.at[i % 2], 11), asbf(w2_i[n]), preferred_element_type=f32)
                g = i * T
                outb_i[n, g // 2:(g + T) // 2, :] = pack(r + hb[i % 2, :, n * 128:(n + 1) * 128])
                if nodma: return
                c = mk(outb.at[n, g:g + T, :], out_hbm.at[g:g + T, n * 128:(n + 1) * 128], sem.at[S_OUT])
                c.start()
                out_started.append(c)
            return f

        L = lambda fn, i, n: [fn(i, c) for c in range(n)] if 0 <= i < NT else []
        Q, A, WO = (lambda i: L(qkv, i, 12)), (lambda i: L(attn, i, NC)), (lambda i: L(wo, i, 4))
        LN1, LN2 = (lambda i: L(ln1, i, NL)), (lambda i: L(ln2, i, NL))
        W1, W2 = (lambda i: L(w1, i, 11)), (lambda i: L(w2, i, 4))
        xwait = lambda i: [wait(X(xg_of[i]))] if i in xg_of else []

        prog = [init]
        if kfine:
            prog += [wait(k_t[0]), wait(k_t[1]), perm_wq(1, 0), wait(X(0))] + LN1(0)
        else:
            prog += [wait(k_t[0], k_t[1]), perm_wq(1, 0), wait(X(0))] + LN1(0)
        prog += [wait(k_t[2], k_t[3]), pinned(perm_wq(1, 1))] + Q(0)[0:4]
        prog += [wait(X(1))] + LN1(1) + pin_at(Q(1)[0:4], pa[1])
        prog += [wait(*v_t), perm_wq(2, 0), perm_wq(2, 1)] + Q(0)[4:8] + pin_at(Q(1)[4:8], pa[2])
        prog += [wait(*q_t), perm_wq(0, 0), perm_wq(0, 1)]
        prog += pin_at(Q(0)[8:12], pa[3]) + [wait(X(2))] + LN1(2) + Q(1)[8:12]
        prog += _interleave(pin_at(Q(2)[0:6], pa[4]), A(0))
        prog += [wait(("wo", 0), ("b1", 0)), prep_b1] + [perm_wo(c) for c in range(4)]
        prog += pin_at(WO(0), pa[5]) + _interleave(Q(2)[6:9], LN2(0))
        w10, w11 = W1(0), pin_at(W1(1), pa[6])
        prog += [wait(("w1a", 0))] + _interleave(pin_at(w10[:w1s], w1s - w1pin), A(1)[:NC // 2])
        prog += [wait(("w1b", 0))] + _interleave(w10[w1s:], A(1)[NC // 2:])
        prog += WO(1) + _interleave(Q(2)[9:12], LN2(1))
        prog += w11[:x3pin] + [wait(("w2", 0)), pinned(W1(1)[x3pin])] + w11[x3pin + 1:]
        prog += xwait(3) + W2(0) + _interleave(W2(1), _interleave(A(2), LN1(3)))
        for i in range(2, NT - 2):
            qn, xw = Q(i + 1), xwait(i + 2)
            prog += WO(i) + _interleave(qn[:qa], LN2(i))
            prog += (pin_at(W1(i), xpin) if xw else W1(i)) + qn[qa:]
            prog += xw + _interleave(W2(i), _interleave(A(i + 1), LN1(i + 2)))
        i = NT - 2
        qn, w2i = Q(i + 1), W2(i)
        prog += WO(i) + _interleave(qn[:qa], LN2(i)) + qn[qa:]
        prog += _interleave(W1(i) + w2i[:4 - hold], A(i + 1))
        prog += WO(i + 1) + _interleave(w2i[4 - hold:], LN2(i + 1)) + W1(i + 1) + W2(i + 1)
        for task in prog:
            task()
        for c in out_started:
            c.wait()

    @jax.jit
    def fn(A_x, A_wqkv, A_wo, B_x, B_w1, B_b1, B_w2):
        hbm = pl.BlockSpec(memory_space=pltpu.HBM)
        out = pl.pallas_call(
            kernel,
            in_specs=[hbm] * 6,
            out_specs=hbm,
            out_shape=jax.ShapeDtypeStruct((S, D), bf16),
            scratch_shapes=[
                pltpu.VMEM((S, D), bf16),
                pltpu.VMEM((12, D, 128), bf16),
                pltpu.VMEM((4, 768, 128), i32),
                pltpu.VMEM((4, D, 128), bf16),
                pltpu.VMEM((4, 256, 128), i32),
                pltpu.VMEM((4, FP, 128), bf16),
                pltpu.VMEM((4, FP, 128), bf16),
                pltpu.VMEM((F,), bf16),
                pltpu.VMEM((8, FP), f32),
                pltpu.VMEM((2, 4, T // 2, 128), i32),
                pltpu.VMEM((4, S, 128), f32),
                pltpu.VMEM((4, S + HALO, 128), f32),
                pltpu.VMEM((4, S + HALO, 128), f32),
                pltpu.VMEM((NT, 4, T // 2, 128), i32),
                pltpu.VMEM((2, T, D), f32),
                pltpu.VMEM((2, 4, T // 2, 128), i32),
                pltpu.VMEM((2, 11, T // 2, 128), i32),
                pltpu.VMEM((4, S, 128), bf16),
                pltpu.VMEM((8, 128), f32),
                pltpu.VMEM((8, 128), i32),
                pltpu.SemaphoreType.DMA((NSEM,)),
            ],
            compiler_params=pltpu.CompilerParams(
                vmem_limit_bytes=64 * 1024 * 1024,
                disable_semaphore_checks=nosc,
                flags={"XLA_TPU_RESCHEDULE_DMA_DONES": True},
            ),
            name="fused_v23",
            interpret=interpret,
        )(A_x.reshape(S, D), A_wqkv, A_wo, B_w1.T, B_b1, B_w2)
        return out.reshape(1, S, D)
    return fn


pallas_sequential_preLN__sliding_local_dilated__dense_activation_mish__prompt_kernel = make()
```

```python
import jax
import jax.numpy as jnp
from jax import lax
import jax.experimental.pallas as pl
import jax.experimental.pallas.tpu as pltpu

S, D, H, DH, F = 2048, 512, 32, 16, 1376
FP = 1408
WIN, DIL = 8, 2
HALO = 16
T = 128
NT = S // T
LOG2E = 1.4426950408889634
f32, bf16, i32 = jnp.float32, jnp.bfloat16, jnp.int32
NT_DIMS = (((1,), (1,)), ((), ()))


def _interleave(a, b):
    out, ia, ib = [], 0, 0
    while ia < len(a) or ib < len(b):
        if ib >= len(b) or (ia < len(a) and (ia + 0.5) * len(b) <= (ib + 0.5) * len(a)):
            out.append(a[ia]); ia += 1
        else:
            out.append(b[ib]); ib += 1
    return out


def make(R=8, LR=16, qa=3, pa=(-1, 1, 0, 1, 0, 2, 3), w1s=5, w1pin=3, xg=(3, 4, 6, 10), xpin=9, x3pin=7,
         hold=2, wopin=2, nosc=True, escpos=5, interpret=False, nodma=False, pins=True):
    xgroups = [(0, 1), (1, 2), (2, xg[0])] + list(zip(xg, list(xg[1:]) + [NT]))
    NX = len(xgroups)
    xg_of = {a: g for g, (a, _) in enumerate(xgroups)}
    S_X, S_W, S_WO, S_B1, S_W1A, S_W1B, S_W2, S_OUT, S_ESC = 0, NX, NX + 12, NX + 13, NX + 14, NX + 15, NX + 16, NX + 17, NX + 18
    NSEM = NX + 19
    W1R = w1s * 128
    NC, NL = T // R, T // LR

    def kernel(x_hbm, wqkv_hbm, wo_hbm, w1t_hbm, b1_hbm, w2_hbm, out_hbm,
               xb, wraw, wq, woraw, wop, w1b, w2b, b1r, bb, xn, qb, kb, vb, ob, hb, hn, act, outb, zf_, zi_, woi, w1p, w2p, sem):
        mk = pltpu.make_async_copy
        asbf = lambda v: pltpu.bitcast(v, bf16)
        pack = lambda v: pltpu.bitcast(v.astype(bf16), i32)

        def copies(nm, z=0):
            kind, idx = nm
            cols = lambda c: slice(c * 128, (c + 1) * 128)
            if kind == "x":
                a, b = xgroups[idx]
                return [mk(x_hbm.at[a * T:b * T, :], xb.at[a * T:b * T, :], sem.at[S_X + idx + z])]
            if kind == "w":
                return [mk(wqkv_hbm.at[:, cols(idx)], wraw.at[idx], sem.at[S_W + idx + z])]
            if kind == "wo":
                return [mk(wo_hbm.at[:, cols(c)], woraw.at[c], sem.at[S_WO + z]) for c in range(4)]
            if kind == "b1":
                return [mk(b1_hbm, b1r, sem.at[S_B1 + z])]
            if kind == "w1a":
                return [mk(w1t_hbm.at[0:W1R, cols(c)], w1b.at[c, 0:W1R, :], sem.at[S_W1A + z]) for c in range(4)]
            if kind == "w1b":
                return [mk(w1t_hbm.at[W1R:F, cols(c)], w1b.at[c, W1R:F, :], sem.at[S_W1B + z]) for c in range(4)]
            if kind == "w2":
                return [mk(w2_hbm.at[:, cols(c)], w2b.at[c, 0:F, :], sem.at[S_W2 + z]) for c in range(4)]

        def start(*names):
            if nodma: return
            for nm in names:
                for c in copies(nm):
                    c.start()

        pin = [0]

        def wait(*names):
            def f():
                z, pin[0] = pin[0], 0
                if nodma: return
                for nm in names:
                    for c in copies(nm, z):
                        c.wait()
            return f

        def pinned(task):
            def f():
                val = task()
                if nodma or not pins: return
                sign = lax.shift_right_logical(pltpu.bitcast(val, i32), 31).astype(f32)
                pin[0] = (jnp.max(sign) * 0.25).astype(i32)
            return f

        def pin_at(tasks, idx):
            return tasks[:idx] + [pinned(tasks[idx])] + tasks[idx + 1:]

        X = lambda g: ("x", g)
        k_t, v_t, q_t = [("w", 4 + a) for a in range(4)], [("w", 8 + a) for a in range(4)], [("w", a) for a in range(4)]
        first = [X(0)] + k_t
        start(*first[:escpos])
        zf_[...] = jnp.zeros((8, 128), f32)
        zi_[...] = jnp.zeros((8, 128), i32)
        esc = [mk(src, dst, sem.at[S_ESC]) for src, dst in (
            (zf_, hb.at[0, 0:8, 0:128]), (zi_, hn.at[0, 0, 0:8, :]), (zi_, act.at[0, 0, 0:8, :]),
            (zi_, xn.at[0, 0, 0:8, :]), (zf_, qb.at[0, 0:8, :]), (zf_, kb.at[0, 0:8, :]), (zf_, vb.at[0, 0:8, :]),
            (zi_, ob.at[0, 0, 0:8, :]), (zi_, wq.at[0, 0:8, :]), (zi_, wop.at[0, 0:8, :]), (zf_, bb.at[:, 0:128]),
            (zi_, woi.at[0, 0:8, :]), (zi_, w1p.at[0, 0:8, :]), (zi_, w2p.at[0, 0:8, :]))]
        for c in esc:
            c.start()
        start(*first[escpos:], X(1), *v_t, *q_t, X(2), ("wo", 0), ("b1", 0), ("w1a", 0), ("w1b", 0), ("w2", 0))
        start(*[X(g) for g in range(3, NX)])
        for c in esc:
            c.wait()

        rr = lax.broadcasted_iota(i32, (128, 128), 0)
        cc = lax.broadcasted_iota(i32, (128, 128), 1)
        P = jnp.where(cc == (rr % 8) * 16 + rr // 8, 1.0, 0.0).astype(bf16)

        def init():
            kb[:, 0:HALO, :] = jnp.zeros((4, HALO, 128), f32)
            vb[:, 0:HALO, :] = jnp.zeros((4, HALO, 128), f32)
            w1b[:, F:FP, :] = jnp.zeros((4, FP - F, 128), bf16)
            w2b[:, F:FP, :] = jnp.zeros((4, FP - F, 128), bf16)

        def perm_wq(part, ap):
            def f():
                rs = [lax.dot_general(P, wraw[part * 4 + a], NT_DIMS, preferred_element_type=f32)
                      for a in (2 * ap, 2 * ap + 1)]
                for d in range(16):
                    pv = pack(jnp.concatenate([rs[0][d * 8:(d + 1) * 8], rs[1][d * 8:(d + 1) * 8]], axis=0))
                    row = (part * D + d * 32 + ap * 16) // 2
                    for kt in range(4):
                        wq[kt, row:row + 8, :] = pv[:, kt * 128:(kt + 1) * 128]
                return rs[1][120:128, 384:512]
            return f

        def perm_wo(c):
            def f():
                woi[c] = pltpu.bitcast(woraw[c], i32)
                for dd in range(8):
                    a = woi[c, pl.ds(dd, 16, stride=16), :]
                    b = woi[c, pl.ds(8 + dd, 16, stride=16), :]
                    wop[c, 32 * dd:32 * dd + 16, :] = (a & 0xFFFF) | lax.shift_left(b, 16)
                    wop[c, 32 * dd + 16:32 * dd + 32, :] = lax.shift_right_logical(a, 16) | (b & jnp.int32(-65536))
            return f

        def prep_b1():
            bb[:, FP - 128:FP] = jnp.zeros((8, 128), f32)
            bb[:, 0:F] = jnp.broadcast_to(b1r[...].astype(f32)[None, :], (8, F))

        def layernorm(xf):
            m = jnp.mean(xf, axis=-1, keepdims=True)
            c = xf - m
            v = jnp.mean(c * c, axis=-1, keepdims=True)
            return c * lax.rsqrt(v + 1e-5)

        def store_lhs(buf, r0, rows, val):
            pv = pack(val)
            for kt in range(val.shape[1] // 128):
                buf[kt, r0 // 2:(r0 + rows) // 2, :] = pv[:, kt * 128:(kt + 1) * 128]

        def load_lhs(buf, nk):
            return jnp.concatenate([asbf(buf[kt]) for kt in range(nk)], axis=1)

        def ln1(i, c):
            def f():
                g = i * T + c * LR
                store_lhs(xn.at[i % 2], c * LR, LR, layernorm(xb[g:g + LR, :].astype(f32)))
            return f

        def qkv(i, n):
            def f():
                part, t = (1, 2, 0)[n // 4], n % 4
                row = (part * D + t * 128) // 2
                rhs = jnp.concatenate([asbf(wq[kt, row:row + 64, :]) for kt in range(4)], axis=1)
                r = lax.dot_general(load_lhs(xn.at[i % 2], 4), rhs, NT_DIMS, preferred_element_type=f32)
                g = i * T
                if part == 0:
                    qb[t, g:g + T, :] = r * (DH ** -0.5 * LOG2E)
                elif part == 1:
                    kb[t, HALO + g:HALO + g + T, :] = r
                else:
                    vb[t, HALO + g:HALO + g + T, :] = r
                return r[T - 8:T, :]
            return f

        def attn(i, c):
            def f():
                g = i * T + c * R
                q = [qb[t, g:g + R, :] for t in range(4)]
                s = []
                for j in range(WIN):
                    a = HALO + g - DIL * j
                    acc = q[0] * kb[0, a:a + R, :]
                    for t in range(1, 4):
                        acc = acc + q[t] * kb[t, a:a + R, :]
                    acc = (acc + pltpu.roll(acc, 64, 1)) + (pltpu.roll(acc, 32, 1) + pltpu.roll(acc, 96, 1))
                    if g < DIL * j:
                        pos = g + lax.broadcasted_iota(i32, (R, 128), 0)
                        acc = jnp.where(pos >= DIL * j, acc, -1e9)
                    s.append(acc)
                m = s[0]
                for j in range(1, WIN):
                    m = jnp.maximum(m, s[j])
                p = [jnp.exp2(sj - m) for sj in s]
                l = p[0]
                for j in range(1, WIN):
                    l = l + p[j]
                inv = pl.reciprocal(l, approx=True)
                o = [None] * 4
                for j in range(WIN):
                    a = HALO + g - DIL * j
                    for t in range(4):
                        term = p[j] * vb[t, a:a + R, :]
                        o[t] = term if o[t] is None else o[t] + term
                for t in range(4):
                    ob[i, t, c * R // 2:(c + 1) * R // 2, :] = pack(o[t] * inv)
            return f

        def wo(i, n):
            def f():
                r = jnp.dot(load_lhs(ob.at[i], 4), asbf(wop[n]), preferred_element_type=f32)
                g = i * T
                hb[i % 2, :, n * 128:(n + 1) * 128] = r + xb[g:g + T, n * 128:(n + 1) * 128].astype(f32)
                return r[T - 8:T, :]
            return f

        def ln2(i, c):
            def f():
                store_lhs(hn.at[i % 2], c * LR, LR, layernorm(hb[i % 2, c * LR:(c + 1) * LR, :]))
            return f

        def w1(i, n):
            def f():
                if i == 0:
                    for kt in range(4):
                        w1p[kt, n * 64:(n + 1) * 64, :] = pltpu.bitcast(w1b[kt, n * 128:(n + 1) * 128, :], i32)
                rhs = jnp.concatenate([asbf(w1p[kt, n * 64:(n + 1) * 64, :]) for kt in range(4)], axis=1)
                h1 = lax.dot_general(load_lhs(hn.at[i % 2], 4), rhs, NT_DIMS, preferred_element_type=f32)
                h1 = h1 + jnp.concatenate([bb[:, n * 128:(n + 1) * 128]] * (T // 8), axis=0)
                e = jnp.exp2(jnp.minimum(h1, 10.0) * LOG2E)
                nn = e * (e + 2.0)
                a = h1 * nn * pl.reciprocal(nn + 2.0, approx=True)
                act[i % 2, n] = pack(a)
                return a[T - 8:T, :]
            return f

        out_started = []

        def w2(i, n):
            def f():
                if i == 0:
                    w2p[n] = pltpu.bitcast(w2b[n], i32)
                r = jnp.dot(load_lhs(act.at[i % 2], 11), asbf(w2p[n]), preferred_element_type=f32)
                g = i * T
                outb[n, g:g + T, :] = (r + hb[i % 2, :, n * 128:(n + 1) * 128]).astype(bf16)
                if nodma: return
                c = mk(outb.at[n, g:g + T, :], out_hbm.at[g:g + T, n * 128:(n + 1) * 128], sem.at[S_OUT])
                c.start()
                out_started.append(c)
            return f

        L = lambda fn, i, n: [fn(i, c) for c in range(n)] if 0 <= i < NT else []
        Q, A, WO = (lambda i: L(qkv, i, 12)), (lambda i: L(attn, i, NC)), (lambda i: L(wo, i, 4))
        LN1, LN2 = (lambda i: L(ln1, i, NL)), (lambda i: L(ln2, i, NL))
        W1, W2 = (lambda i: L(w1, i, 11)), (lambda i: L(w2, i, 4))
        xwait = lambda i: [wait(X(xg_of[i]))] if i in xg_of else []

        prog = [init]
        prog += [wait(k_t[0], k_t[1]), perm_wq(1, 0), wait(X(0))] + LN1(0)
        prog += [wait(k_t[2], k_t[3]), pinned(perm_wq(1, 1))] + Q(0)[0:4]
        prog += [wait(X(1))] + LN1(1) + pin_at(Q(1)[0:4], pa[1])
        prog += [wait(*v_t), perm_wq(2, 0), perm_wq(2, 1)] + Q(0)[4:8] + pin_at(Q(1)[4:8], pa[2])
        prog += [wait(*q_t), perm_wq(0, 0), perm_wq(0, 1)]
        prog += pin_at(Q(0)[8:12], pa[3]) + [wait(X(2))] + LN1(2) + pin_at(Q(1)[8:12], wopin)
        prog += [wait(("wo", 0), ("b1", 0)), prep_b1] + [perm_wo(c) for c in range(4)]
        prog += _interleave(Q(2)[0:6], A(0))
        prog += pin_at(WO(0), pa[5]) + _interleave(Q(2)[6:9], LN2(0))
        w10, w11 = W1(0), pin_at(W1(1), pa[6])
        prog += [wait(("w1a", 0))] + _interleave(pin_at(w10[:w1s], w1s - w1pin), A(1)[:NC // 2])
        prog += [wait(("w1b", 0))] + _interleave(w10[w1s:], A(1)[NC // 2:])
        prog += WO(1) + _interleave(Q(2)[9:12], LN2(1))
        prog += w11[:x3pin] + [wait(("w2", 0)), pinned(W1(1)[x3pin])] + w11[x3pin + 1:]
        prog += xwait(3) + W2(0) + _interleave(W2(1), _interleave(A(2), LN1(3)))
        for i in range(2, NT - 2):
            qn, xw = Q(i + 1), xwait(i + 2)
            prog += WO(i) + _interleave(qn[:qa], LN2(i))
            prog += (pin_at(W1(i), xpin) if xw else W1(i)) + qn[qa:]
            prog += xw + _interleave(W2(i), _interleave(A(i + 1), LN1(i + 2)))
        i = NT - 2
        qn, w2i = Q(i + 1), W2(i)
        prog += WO(i) + _interleave(qn[:qa], LN2(i)) + qn[qa:]
        prog += _interleave(W1(i) + w2i[:4 - hold], A(i + 1))
        prog += WO(i + 1) + _interleave(w2i[4 - hold:], LN2(i + 1)) + W1(i + 1) + W2(i + 1)
        for task in prog:
            task()
        for c in out_started:
            c.wait()

    @jax.jit
    def fn(A_x, A_wqkv, A_wo, B_x, B_w1, B_b1, B_w2):
        hbm = pl.BlockSpec(memory_space=pltpu.HBM)
        out = pl.pallas_call(
            kernel,
            in_specs=[hbm] * 6,
            out_specs=hbm,
            out_shape=jax.ShapeDtypeStruct((S, D), bf16),
            scratch_shapes=[
                pltpu.VMEM((S, D), bf16),
                pltpu.VMEM((12, D, 128), bf16),
                pltpu.VMEM((4, 768, 128), i32),
                pltpu.VMEM((4, D, 128), bf16),
                pltpu.VMEM((4, 256, 128), i32),
                pltpu.VMEM((4, FP, 128), bf16),
                pltpu.VMEM((4, FP, 128), bf16),
                pltpu.VMEM((F,), bf16),
                pltpu.VMEM((8, FP), f32),
                pltpu.VMEM((2, 4, T // 2, 128), i32),
                pltpu.VMEM((4, S, 128), f32),
                pltpu.VMEM((4, S + HALO, 128), f32),
                pltpu.VMEM((4, S + HALO, 128), f32),
                pltpu.VMEM((NT, 4, T // 2, 128), i32),
                pltpu.VMEM((2, T, D), f32),
                pltpu.VMEM((2, 4, T // 2, 128), i32),
                pltpu.VMEM((2, 11, T // 2, 128), i32),
                pltpu.VMEM((4, S, 128), bf16),
                pltpu.VMEM((8, 128), f32),
                pltpu.VMEM((8, 128), i32),
                pltpu.VMEM((4, 256, 128), i32),
                pltpu.VMEM((4, FP // 2, 128), i32),
                pltpu.VMEM((4, FP // 2, 128), i32),
                pltpu.SemaphoreType.DMA((NSEM,)),
            ],
            compiler_params=pltpu.CompilerParams(
                vmem_limit_bytes=64 * 1024 * 1024,
                disable_semaphore_checks=nosc,
                flags={"XLA_TPU_RESCHEDULE_DMA_DONES": True},
            ),
            name="fused_block",
            interpret=interpret,
        )(A_x.reshape(S, D), A_wqkv, A_wo, B_w1.T, B_b1, B_w2)
        return out.reshape(1, S, D)
    return fn


pallas_sequential_preLN__sliding_local_dilated__dense_activation_mish__prompt_kernel = make()
```

```python
import jax
import jax.numpy as jnp
from jax import lax
import jax.experimental.pallas as pl
import jax.experimental.pallas.tpu as pltpu

S, D, H, DH, F = 2048, 512, 32, 16, 1376
FP = 1408
WIN, DIL = 8, 2
HALO = 16
T = 128
NT = S // T
R, LR = 8, 16
NC, NL = T // R, T // LR
W1R = 5 * 128
LOG2E = 1.4426950408889634
f32, bf16, i32 = jnp.float32, jnp.bfloat16, jnp.int32
NT_DIMS = (((1,), (1,)), ((), ()))

X_GROUPS = ((0, 1), (1, 2), (2, 3), (3, 4), (4, 6), (6, 10), (10, 16))
NX = len(X_GROUPS)
X_GROUP_AT = {a: g for g, (a, _) in enumerate(X_GROUPS)}
S_X, S_W, S_WO, S_B1, S_W1A, S_W1B, S_W2, S_OUT, S_ESC = (
    0, NX, NX + 12, NX + 13, NX + 14, NX + 15, NX + 16, NX + 17, NX + 18)
NSEM = NX + 19


def _interleave(a, b):
    out, ia, ib = [], 0, 0
    while ia < len(a) or ib < len(b):
        if ib >= len(b) or (ia < len(a) and (ia + 0.5) * len(b) <= (ib + 0.5) * len(a)):
            out.append(a[ia]); ia += 1
        else:
            out.append(b[ib]); ib += 1
    return out


def _kernel(x_hbm, wqkv_hbm, wo_hbm, w1t_hbm, b1_hbm, w2_hbm, out_hbm,
            xb, wraw, wq, woraw, wop, w1b, w2b, b1r, bb,
            xn, qb, kb, vb, ob, hb, hn, act, outb, zf, zi, woi, w1p, w2p, sem):
    mk = pltpu.make_async_copy
    asbf = lambda v: pltpu.bitcast(v, bf16)
    pack = lambda v: pltpu.bitcast(v.astype(bf16), i32)
    cols = lambda c: slice(c * 128, (c + 1) * 128)

    def copies(name, z=0):
        kind, idx = name
        if kind == "x":
            a, b = X_GROUPS[idx]
            return [mk(x_hbm.at[a * T:b * T, :], xb.at[a * T:b * T, :], sem.at[S_X + idx + z])]
        if kind == "w":
            return [mk(wqkv_hbm.at[:, cols(idx)], wraw.at[idx], sem.at[S_W + idx + z])]
        if kind == "wo":
            return [mk(wo_hbm.at[:, cols(c)], woraw.at[c], sem.at[S_WO + z]) for c in range(4)]
        if kind == "b1":
            return [mk(b1_hbm, b1r, sem.at[S_B1 + z])]
        if kind == "w1a":
            return [mk(w1t_hbm.at[0:W1R, cols(c)], w1b.at[c, 0:W1R, :], sem.at[S_W1A + z]) for c in range(4)]
        if kind == "w1b":
            return [mk(w1t_hbm.at[W1R:F, cols(c)], w1b.at[c, W1R:F, :], sem.at[S_W1B + z]) for c in range(4)]
        if kind == "w2":
            return [mk(w2_hbm.at[:, cols(c)], w2b.at[c, 0:F, :], sem.at[S_W2 + z]) for c in range(4)]

    def start(*names):
        for name in names:
            for c in copies(name):
                c.start()

    pin = [0]

    def wait(*names):
        def f():
            z, pin[0] = pin[0], 0
            for name in names:
                for c in copies(name, z):
                    c.wait()
        return f

    def pinned(task):
        def f():
            val = task()
            sign = lax.shift_right_logical(pltpu.bitcast(val, i32), 31).astype(f32)
            pin[0] = (jnp.max(sign) * 0.25).astype(i32)
        return f

    def pin_at(tasks, idx):
        return tasks[:idx] + [pinned(tasks[idx])] + tasks[idx + 1:]

    X = lambda g: ("x", g)
    k_t, v_t, q_t = ([("w", 4 * part + a) for a in range(4)] for part in (1, 2, 0))
    start(X(0), *k_t)
    zf[...] = jnp.zeros((8, 128), f32)
    zi[...] = jnp.zeros((8, 128), i32)
    keep = [mk(src, dst, sem.at[S_ESC]) for src, dst in (
        (zf, hb.at[0, 0:8, 0:128]), (zi, hn.at[0, 0, 0:8, :]), (zi, act.at[0, 0, 0:8, :]),
        (zi, xn.at[0, 0, 0:8, :]), (zf, qb.at[0, 0:8, :]), (zf, kb.at[0, 0:8, :]), (zf, vb.at[0, 0:8, :]),
        (zi, ob.at[0, 0, 0:8, :]), (zi, wq.at[0, 0:8, :]), (zi, wop.at[0, 0:8, :]), (zf, bb.at[:, 0:128]),
        (zi, woi.at[0, 0:8, :]), (zi, w1p.at[0, 0:8, :]), (zi, w2p.at[0, 0:8, :]))]
    for c in keep:
        c.start()
    start(X(1), *v_t, *q_t, X(2), ("wo", 0), ("b1", 0), ("w1a", 0), ("w1b", 0), ("w2", 0))
    start(*[X(g) for g in range(3, NX)])
    for c in keep:
        c.wait()

    rr = lax.broadcasted_iota(i32, (128, 128), 0)
    cc = lax.broadcasted_iota(i32, (128, 128), 1)
    P = jnp.where(cc == (rr % 8) * 16 + rr // 8, 1.0, 0.0).astype(bf16)

    def init():
        kb[:, 0:HALO, :] = jnp.zeros((4, HALO, 128), f32)
        vb[:, 0:HALO, :] = jnp.zeros((4, HALO, 128), f32)
        w1b[:, F:FP, :] = jnp.zeros((4, FP - F, 128), bf16)
        w2b[:, F:FP, :] = jnp.zeros((4, FP - F, 128), bf16)

    def perm_wq(part, ap):
        def f():
            rs = [lax.dot_general(P, wraw[part * 4 + a], NT_DIMS, preferred_element_type=f32)
                  for a in (2 * ap, 2 * ap + 1)]
            for d in range(16):
                pv = pack(jnp.concatenate([rs[0][d * 8:(d + 1) * 8], rs[1][d * 8:(d + 1) * 8]], axis=0))
                row = (part * D + d * 32 + ap * 16) // 2
                for kt in range(4):
                    wq[kt, row:row + 8, :] = pv[:, cols(kt)]
            return rs[1][120:128, 384:512]
        return f

    def perm_wo(c):
        def f():
            woi[c] = pltpu.bitcast(woraw[c], i32)
            for dd in range(8):
                a = woi[c, pl.ds(dd, 16, stride=16), :]
                b = woi[c, pl.ds(8 + dd, 16, stride=16), :]
                wop[c, 32 * dd:32 * dd + 16, :] = (a & 0xFFFF) | lax.shift_left(b, 16)
                wop[c, 32 * dd + 16:32 * dd + 32, :] = lax.shift_right_logical(a, 16) | (b & jnp.int32(-65536))
        return f

    def prep_b1():
        bb[:, FP - 128:FP] = jnp.zeros((8, 128), f32)
        bb[:, 0:F] = jnp.broadcast_to(b1r[...].astype(f32)[None, :], (8, F))

    def layernorm(xf):
        m = jnp.mean(xf, axis=-1, keepdims=True)
        c = xf - m
        v = jnp.mean(c * c, axis=-1, keepdims=True)
        return c * lax.rsqrt(v + 1e-5)

    def store_lhs(buf, r0, val):
        pv = pack(val)
        for kt in range(val.shape[1] // 128):
            buf[kt, r0 // 2:(r0 + val.shape[0]) // 2, :] = pv[:, cols(kt)]

    def load_lhs(buf, nk):
        return jnp.concatenate([asbf(buf[kt]) for kt in range(nk)], axis=1)

    def ln1(i, c):
        def f():
            g = i * T + c * LR
            store_lhs(xn.at[i % 2], c * LR, layernorm(xb[g:g + LR, :].astype(f32)))
        return f

    def qkv(i, n):
        def f():
            part, t = (1, 2, 0)[n // 4], n % 4
            row = (part * D + t * 128) // 2
            rhs = jnp.concatenate([asbf(wq[kt, row:row + 64, :]) for kt in range(4)], axis=1)
            r = lax.dot_general(load_lhs(xn.at[i % 2], 4), rhs, NT_DIMS, preferred_element_type=f32)
            g = i * T
            if part == 0:
                qb[t, g:g + T, :] = r * (DH ** -0.5 * LOG2E)
            elif part == 1:
                kb[t, HALO + g:HALO + g + T, :] = r
            else:
                vb[t, HALO + g:HALO + g + T, :] = r
            return r[T - 8:T, :]
        return f

    def attn(i, c):
        def f():
            g = i * T + c * R
            q = [qb[t, g:g + R, :] for t in range(4)]
            s = []
            for j in range(WIN):
                a = HALO + g - DIL * j
                acc = q[0] * kb[0, a:a + R, :]
                for t in range(1, 4):
                    acc = acc + q[t] * kb[t, a:a + R, :]
                acc = (acc + pltpu.roll(acc, 64, 1)) + (pltpu.roll(acc, 32, 1) + pltpu.roll(acc, 96, 1))
                if g < DIL * j:
                    pos = g + lax.broadcasted_iota(i32, (R, 128), 0)
                    acc = jnp.where(pos >= DIL * j, acc, -1e9)
                s.append(acc)
            m = s[0]
            for j in range(1, WIN):
                m = jnp.maximum(m, s[j])
            p = [jnp.exp2(sj - m) for sj in s]
            l = p[0]
            for j in range(1, WIN):
                l = l + p[j]
            inv = pl.reciprocal(l, approx=True)
            o = [None] * 4
            for j in range(WIN):
                a = HALO + g - DIL * j
                for t in range(4):
                    term = p[j] * vb[t, a:a + R, :]
                    o[t] = term if o[t] is None else o[t] + term
            for t in range(4):
                ob[i, t, c * R // 2:(c + 1) * R // 2, :] = pack(o[t] * inv)
        return f

    def wo(i, n):
        def f():
            r = jnp.dot(load_lhs(ob.at[i], 4), asbf(wop[n]), preferred_element_type=f32)
            g = i * T
            hb[i % 2, :, cols(n)] = r + xb[g:g + T, cols(n)].astype(f32)
            return r[T - 8:T, :]
        return f

    def ln2(i, c):
        def f():
            store_lhs(hn.at[i % 2], c * LR, layernorm(hb[i % 2, c * LR:(c + 1) * LR, :]))
        return f

    def w1(i, n):
        def f():
            if i == 0:
                for kt in range(4):
                    w1p[kt, n * 64:(n + 1) * 64, :] = pltpu.bitcast(w1b[kt, n * 128:(n + 1) * 128, :], i32)
            rhs = jnp.concatenate([asbf(w1p[kt, n * 64:(n + 1) * 64, :]) for kt in range(4)], axis=1)
            h1 = lax.dot_general(load_lhs(hn.at[i % 2], 4), rhs, NT_DIMS, preferred_element_type=f32)
            h1 = h1 + jnp.concatenate([bb[:, cols(n)]] * (T // 8), axis=0)
            e = jnp.exp2(jnp.minimum(h1, 10.0) * LOG2E)
            nn = e * (e + 2.0)
            a = h1 * nn * pl.reciprocal(nn + 2.0, approx=True)
            act[i % 2, n] = pack(a)
            return a[T - 8:T, :]
        return f

    out_copies = []

    def w2(i, n):
        def f():
            if i == 0:
                w2p[n] = pltpu.bitcast(w2b[n], i32)
            r = jnp.dot(load_lhs(act.at[i % 2], 11), asbf(w2p[n]), preferred_element_type=f32)
            g = i * T
            outb[n, g:g + T, :] = (r + hb[i % 2, :, cols(n)]).astype(bf16)
            c = mk(outb.at[n, g:g + T, :], out_hbm.at[g:g + T, cols(n)], sem.at[S_OUT])
            c.start()
            out_copies.append(c)
        return f

    L = lambda fn, i, n: [fn(i, c) for c in range(n)]
    Q, A, WO = (lambda i: L(qkv, i, 12)), (lambda i: L(attn, i, NC)), (lambda i: L(wo, i, 4))
    LN1, LN2 = (lambda i: L(ln1, i, NL)), (lambda i: L(ln2, i, NL))
    W1, W2 = (lambda i: L(w1, i, 11)), (lambda i: L(w2, i, 4))
    xwait = lambda i: [wait(X(X_GROUP_AT[i]))] if i in X_GROUP_AT else []

    prog = [init]
    prog += [wait(k_t[0], k_t[1]), perm_wq(1, 0), wait(X(0))] + LN1(0)
    prog += [wait(k_t[2], k_t[3]), pinned(perm_wq(1, 1))] + Q(0)[0:4]
    prog += [wait(X(1))] + LN1(1) + pin_at(Q(1)[0:4], 1)
    prog += [wait(*v_t), perm_wq(2, 0), perm_wq(2, 1)] + Q(0)[4:8] + pin_at(Q(1)[4:8], 0)
    prog += [wait(*q_t), perm_wq(0, 0), perm_wq(0, 1)]
    prog += pin_at(Q(0)[8:12], 1) + [wait(X(2))] + LN1(2) + pin_at(Q(1)[8:12], 2)
    prog += [wait(("wo", 0), ("b1", 0)), prep_b1] + [perm_wo(c) for c in range(4)]
    prog += _interleave(Q(2)[0:6], A(0))
    prog += pin_at(WO(0), 2) + _interleave(Q(2)[6:9], LN2(0))
    w10, w11 = W1(0), pin_at(W1(1), 3)
    prog += [wait(("w1a", 0))] + _interleave(pin_at(w10[:5], 2), A(1)[:NC // 2])
    prog += [wait(("w1b", 0))] + _interleave(w10[5:], A(1)[NC // 2:])
    prog += WO(1) + _interleave(Q(2)[9:12], LN2(1))
    prog += w11[:7] + [wait(("w2", 0)), pinned(W1(1)[7])] + w11[8:]
    prog += xwait(3) + W2(0) + _interleave(W2(1), _interleave(A(2), LN1(3)))
    for i in range(2, NT - 2):
        qn, xw = Q(i + 1), xwait(i + 2)
        prog += WO(i) + _interleave(qn[:3], LN2(i))
        prog += (pin_at(W1(i), 9) if xw else W1(i)) + qn[3:]
        prog += xw + _interleave(W2(i), _interleave(A(i + 1), LN1(i + 2)))
    i = NT - 2
    qn, w2i = Q(i + 1), W2(i)
    prog += WO(i) + _interleave(qn[:3], LN2(i)) + qn[3:]
    prog += _interleave(W1(i) + w2i[:2], A(i + 1))
    prog += WO(i + 1) + _interleave(w2i[2:], LN2(i + 1)) + W1(i + 1) + W2(i + 1)
    for task in prog:
        task()
    for c in out_copies:
        c.wait()


@jax.jit
def pallas_sequential_preLN__sliding_local_dilated__dense_activation_mish__prompt_kernel(
    A_x: jax.Array,
    A_wqkv: jax.Array,
    A_wo: jax.Array,
    B_x: jax.Array,
    B_w1: jax.Array,
    B_b1: jax.Array,
    B_w2: jax.Array,
):
    hbm = pl.BlockSpec(memory_space=pltpu.HBM)
    out = pl.pallas_call(
        _kernel,
        in_specs=[hbm] * 6,
        out_specs=hbm,
        out_shape=jax.ShapeDtypeStruct((S, D), bf16),
        scratch_shapes=[
            pltpu.VMEM((S, D), bf16),
            pltpu.VMEM((12, D, 128), bf16),
            pltpu.VMEM((4, 768, 128), i32),
            pltpu.VMEM((4, D, 128), bf16),
            pltpu.VMEM((4, D // 2, 128), i32),
            pltpu.VMEM((4, FP, 128), bf16),
            pltpu.VMEM((4, FP, 128), bf16),
            pltpu.VMEM((F,), bf16),
            pltpu.VMEM((8, FP), f32),
            pltpu.VMEM((2, 4, T // 2, 128), i32),
            pltpu.VMEM((4, S, 128), f32),
            pltpu.VMEM((4, S + HALO, 128), f32),
            pltpu.VMEM((4, S + HALO, 128), f32),
            pltpu.VMEM((NT, 4, T // 2, 128), i32),
            pltpu.VMEM((2, T, D), f32),
            pltpu.VMEM((2, 4, T // 2, 128), i32),
            pltpu.VMEM((2, 11, T // 2, 128), i32),
            pltpu.VMEM((4, S, 128), bf16),
            pltpu.VMEM((8, 128), f32),
            pltpu.VMEM((8, 128), i32),
            pltpu.VMEM((4, D // 2, 128), i32),
            pltpu.VMEM((4, FP // 2, 128), i32),
            pltpu.VMEM((4, FP // 2, 128), i32),
            pltpu.SemaphoreType.DMA((NSEM,)),
        ],
        compiler_params=pltpu.CompilerParams(
            vmem_limit_bytes=64 * 1024 * 1024,
            disable_semaphore_checks=True,
            flags={"XLA_TPU_RESCHEDULE_DMA_DONES": True},
        ),
        name="fused_block",
    )(A_x.reshape(S, D), A_wqkv, A_wo, B_w1.T, B_b1, B_w2)
    return out.reshape(1, S, D)
```
